```python
import os as _os
_os.environ.setdefault("JAX_PLATFORMS", "cpu")
import jax
import jax.numpy as jnp

def _softmax(x, axis=-1):
    return jax.nn.softmax(x, axis=axis)
def _gelu(x):
    return jax.nn.gelu(x, approximate=True)
def _silu(x):
    return jax.nn.silu(x)
def _sigmoid(x):
    return jax.nn.sigmoid(x)
def _layernorm(x, axis=-1, eps=1e-5):
    m = jnp.mean(x, axis=axis, keepdims=True)
    v = jnp.var(x, axis=axis, keepdims=True)
    return (x - m) / jnp.sqrt(v + eps)
def _scatter_add(tgt, idx, src, axis=0):
    return tgt.at[idx].add(src)
def _segment_sum(src, seg, n):
    return jax.ops.segment_sum(src, seg, n)
class _Rng:
    def __init__(self, key):
        self._k = key
    def _next(self):
        self._k, sub = jax.random.split(self._k)
        return sub
    def normal(self, shape):
        return jax.random.normal(self._next(), shape, dtype=jnp.bfloat16)
    def randint(self, lo, hi, shape):
        return jax.random.randint(self._next(), shape, lo, hi, dtype=jnp.int32)
    def uniform(self, shape, lo=0.0, hi=1.0):
        return jax.random.uniform(self._next(), shape, jnp.bfloat16, lo, hi)
    def permutation(self, n):
        return jax.random.permutation(self._next(), n)


kernel_name = 'concat_heads__sliding_block_cached__mha_block_cached__decode'

def setup_inputs():
    _rng = _Rng(jax.random.key(int.from_bytes(__import__("os").urandom(4), "little")))
    _w = (lambda a: (lambda t: t.astype(jnp.bfloat16) if jnp.issubdtype(t.dtype, jnp.floating) else t)(jnp.asarray(a)))
    def _A_setup():
        B, Sq, D = 4, 1, 640
        Hq, Hkv, Sk, Dh = 32, 32, 4096, 128
        assert Hq % Hkv == 0, (Hq, Hkv)
        return {
            "x": _w((lambda *s: _rng.normal(s) * 0.8)(B, Sq, D)),
            "k_cache": _w((lambda *s: _rng.normal(s) * 0.8)(B, Hkv, Sk, Dh)),
            "v_cache": _w((lambda *s: _rng.normal(s) * 0.05)(B, Hkv, Sk, Dh)),
            "wq": _w((lambda *s: _rng.normal(s) * 0.8)(D, Hq * Dh) * (D ** -0.5)),
            "wo": _w((lambda *s: _rng.normal(s) * 0.05)(Hq * Dh, D) * ((Hq * Dh) ** -0.5)),
        }
    _A_in = _A_setup()

    def _B_setup():
        B, Sq, D = 4, 1, 640
        H, Sk, Dh = 32, 4096, 128
        return {
            "x": _w((lambda *s: _rng.normal(s) * 0.8)(B, Sq, D)),
            "k_cache": _w((lambda *s: _rng.normal(s) * 0.8)(B, H, Sk, Dh)),
            "v_cache": _w((lambda *s: _rng.normal(s) * 0.05)(B, H, Sk, Dh)),
            "wq": _w((lambda *s: _rng.normal(s) * 0.8)(D, H * Dh) * (D ** -0.5)),
            "wo": _w((lambda *s: _rng.normal(s) * 0.05)(H * Dh, D) * ((H * Dh) ** -0.5)),
        }
    _B_in = _B_setup()

    return {
        "A_x": _A_in["x"],
        "A_k_cache": _A_in["k_cache"],
        "A_v_cache": _A_in["v_cache"],
        "A_wq": _A_in["wq"],
        "A_wo": _A_in["wo"],
        "B_x": _B_in["x"],
        "B_k_cache": _B_in["k_cache"],
        "B_v_cache": _B_in["v_cache"],
        "B_wq": _B_in["wq"],
        "B_wo": _B_in["wo"],
    }

def reference(A_x, A_k_cache, A_v_cache, A_wq, A_wo, B_x, B_k_cache, B_v_cache, B_wq, B_wo):
    def _A_ref(x, k_cache, v_cache, wq, wo):
        B, Sq, D = x.shape
        Hq, Dh = 32, 128
        Hkv, Sk = k_cache.shape[1], k_cache.shape[2]
        W = min(4096, max(256, Sk // 4))
        rep = Hq // Hkv
        q = (lambda x, *d: x.transpose(*d))((x @ wq).reshape(B, Sq, Hq, Dh), 0, 2, 1, 3)
        k = jnp.repeat(k_cache[:, :, Sk - W:, :], rep, axis=1)
        v = jnp.repeat(v_cache[:, :, Sk - W:, :], rep, axis=1)
        scores = jnp.einsum("bhqd,bhkd->bhqk", q, k) * (Dh ** -0.5)
        p = _softmax(scores, axis=-1)
        o = jnp.einsum("bhqk,bhkd->bhqd", p, v)
        return (lambda x, *d: x.transpose(*d))(o, 0, 2, 1, 3).reshape(B, Sq, Hq * Dh) @ wo

    def _B_ref(x, k_cache, v_cache, wq, wo):
        B, Sq, D = x.shape
        H, Dh = 32, 128
        q = (lambda x, *d: x.transpose(*d))((x @ wq).reshape(B, Sq, H, Dh), 0, 2, 1, 3)
        scores = jnp.einsum("bhqd,bhkd->bhqk", q, k_cache) * (Dh ** -0.5)
        p = _softmax(scores, axis=-1)
        o = jnp.einsum("bhqk,bhkd->bhqd", p, v_cache)
        return (lambda x, *d: x.transpose(*d))(o, 0, 2, 1, 3).reshape(B, Sq, H * Dh) @ wo

    a = _A_ref(A_x, A_k_cache, A_v_cache, A_wq, A_wo)
    b = _B_ref(B_x, B_k_cache, B_v_cache, B_wq, B_wo)
    return jnp.concatenate([a, b], axis=-1)
```

```python
import functools

import jax
import jax.numpy as jnp
import jax.experimental.pallas as pl
import jax.experimental.pallas.tpu as pltpu

G = 8
R = 128
DH = 128
NSLOT = 16
LA = 8
NLOW = 7
NPIECE = 4


def _kernel(xa_hbm, ka_hbm, va_hbm, wqa_hbm, woa_hbm,
            xb_hbm, kb_hbm, vb_hbm, wqb_hbm, wob_hbm,
            out_ref,
            buf, xa_v, xb_v, wqa_v, wqb_v, woa_v, wob_v,
            qt_v, q_v, s_v, o_v, acc_v,
            sem, xsem, wqsem, wosem,
            *, nb, nh, sk, wa):
    f32 = jnp.float32
    bf16 = jnp.bfloat16
    ngrp = nh // G
    nstep = ngrp * nb
    dmodel = xa_v.shape[-1]
    gcols = G * DH
    scale = DH ** -0.5
    ta = wa // R
    tb = sk // R
    a_row0 = sk - wa
    prow = R // NPIECE
    rowid = jax.lax.broadcasted_iota(jnp.int32, (G, DH), 0)

    def chunk_copies(src, b, g, row0, slot):
        low = pltpu.make_async_copy(
            src.at[b, pl.ds(g * G, NLOW), pl.ds(row0, R)],
            buf.at[slot, pl.ds(0, NLOW)], sem.at[slot])
        high = []
        for hh in range(NLOW, G):
            for u in range(NPIECE):
                high.append(pltpu.make_async_copy(
                    src.at[b, g * G + hh, pl.ds(row0 + u * prow, prow)],
                    buf.at[slot, hh, pl.ds(u * prow, prow)], sem.at[slot]))
        return low, high

    def chunk_wait(slot):
        pltpu.make_async_copy(buf.at[slot], buf.at[slot], sem.at[slot]).wait()

    def diag(parts):
        out = parts[0]
        for r in range(1, G):
            out = jnp.where(rowid == r, parts[r], out)
        return out

    def tick(tau, nxt, extra, tile_fn):
        slot = tau % NSLOT
        starts = []
        if nxt is not None:
            src, b, g, row0, cond = nxt
            low, high = chunk_copies(src, b, g, row0, (tau + LA) % NSLOT)
            starts = [(low, 1, cond)] + [(h, 0, cond) for h in high]
        starts = starts + extra

        def do_start(item):
            cp, prio, cond = item
            if cond is None:
                cp.start(priority=prio)
            else:
                @pl.when(cond)
                def _():
                    cp.start(priority=prio)

        chunk_wait(slot)
        parts = []
        n = len(starts)
        done = 0
        for r in range(G):
            want = min(n, 2 + (r * n) // G) if n else 0
            while done < want:
                do_start(starts[done])
                done += 1
            parts.append(tile_fn(buf[slot, r]))
        while done < n:
            do_start(starts[done])
            done += 1
        return diag(parts)

    def k_phase(tau0, t0, nt, q, m, nxt_fn, extra_fn):
        def body(t, m):
            s = tick(tau0 + t, nxt_fn(t), extra_fn(t),
                     lambda k: jax.lax.dot_general(
                         q, k, (((1,), (1,)), ((), ())),
                         preferred_element_type=f32))
            s_v[t] = s
            return jnp.maximum(m, s)
        return jax.lax.fori_loop(t0, t0 + nt, body, m)

    def v_phase(tau0, t0, nt, mrow, carry, nxt_fn, extra_fn):
        def body(t, carry):
            l, acc = carry
            p = jnp.exp((s_v[t] - mrow) * scale)
            pb = p.astype(bf16)
            o = tick(tau0 + t, nxt_fn(t), extra_fn(t),
                     lambda v: jnp.dot(pb, v, preferred_element_type=f32))
            return l + p, acc + o
        return jax.lax.fori_loop(t0, t0 + nt, body, carry)

    no_extra = lambda t: []

    wq_rows = 16
    wq_per_step = dmodel // wq_rows // nb
    wo_rows = gcols // nb // 8

    def wq_piece(w_hbm, w_v, which, g, idx):
        return pltpu.make_async_copy(
            w_hbm.at[pl.ds(idx * wq_rows, wq_rows), pl.ds(g * gcols, gcols)],
            w_v.at[g, pl.ds(idx * wq_rows, wq_rows)], wqsem.at[which, g])

    def wo_piece(w_hbm, w_v, which, g, idx):
        return pltpu.make_async_copy(
            w_hbm.at[pl.ds(g * gcols + idx * wo_rows, wo_rows)],
            w_v.at[g, pl.ds(idx * wo_rows, wo_rows)], wosem.at[which, g])

    def q_proj(which, x_v, w_v, g):
        pltpu.make_async_copy(w_v.at[g], w_v.at[g], wqsem.at[which, g]).wait()
        x = x_v[...]
        q = jnp.dot(x, w_v[g], preferred_element_type=f32)
        for r in range(G):
            qt_v[pl.ds(r * 8, nb), :] = q[:, r * DH:(r + 1) * DH]
        for b in range(nb):
            q_v[which, b] = qt_v[pl.ds(b, G, stride=8), :].astype(bf16).astype(f32)

    def out_proj(which, w_v, g):
        pltpu.make_async_copy(w_v.at[g], w_v.at[g], wosem.at[which, g]).wait()
        o = jnp.concatenate(
            [o_v[which, pl.ds(r, nb, stride=G), :] for r in range(G)], axis=1)
        acc_v[which] += jnp.dot(o.astype(bf16), w_v[g],
                                preferred_element_type=f32)

    pltpu.make_async_copy(wqa_hbm.at[:, pl.ds(0, gcols)], wqa_v.at[0],
                          wqsem.at[0, 0]).start(priority=0)
    xa_cp = pltpu.make_async_copy(xa_hbm, xa_v, xsem.at[0])
    xb_cp = pltpu.make_async_copy(xb_hbm, xb_v, xsem.at[1])
    xa_cp.start(priority=0)
    xb_cp.start(priority=0)
    for t in range(LA):
        low, _ = chunk_copies(ka_hbm, 0, 0, a_row0 + t * R, t)
        low.start(priority=1)
    pltpu.make_async_copy(wqb_hbm.at[:, pl.ds(0, gcols)], wqb_v.at[0],
                          wqsem.at[1, 0]).start(priority=0)
    for t in range(LA):
        _, high = chunk_copies(ka_hbm, 0, 0, a_row0 + t * R, t)
        for h in high:
            h.start(priority=0)
    acc_v[...] = jnp.zeros(acc_v.shape, f32)
    xa_cp.wait()
    xb_cp.wait()

    def step(i, c):
        g = i // nb
        b = i % nb
        i2 = jnp.minimum(i + 1, nstep - 1)
        g2 = i2 // nb
        b2 = i2 % nb
        gw = jnp.minimum(g + 1, ngrp - 1)

        @pl.when(b == 0)
        def _():
            q_proj(0, xa_v, wqa_v, g)
            q_proj(1, xb_v, wqb_v, g)

        neg = jnp.full((G, DH), -jnp.inf, f32)
        zero = jnp.zeros((G, DH), f32)

        def finish(which, carry):
            l, acc = carry
            lsum = jnp.sum(l, axis=1, keepdims=True)
            o_v[which, pl.ds(pl.multiple_of(b * G, G), G), :] = acc / lsum

        qa = q_v[0, b].astype(bf16)
        m = k_phase(0, 0, ta, qa, neg,
                    lambda t: (va_hbm, b, g, a_row0 + t * R, None), no_extra)
        mrow = jnp.max(m, axis=1, keepdims=True)
        carry = v_phase(ta, 0, ta, mrow, (zero, zero),
                        lambda t: (kb_hbm, b, g, t * R, None), no_extra)
        finish(0, carry)

        tau0 = 2 * ta
        qb = q_v[1, b].astype(bf16)
        nk = lambda t: (kb_hbm, b, g, (t + LA) * R, None)
        m = k_phase(tau0, 0, 8, qb, neg, nk,
                    lambda t: [(wo_piece(woa_hbm, woa_v, 0, g, b * 8 + t), 0, None),
                               (wo_piece(wob_hbm, wob_v, 1, g, b * 8 + t), 0, None)])
        m = k_phase(tau0, 8, tb - LA - 8, qb, m, nk, no_extra)
        m = k_phase(tau0, tb - LA, LA, qb, m,
                    lambda t: (vb_hbm, b, g, (t + LA - tb) * R, None), no_extra)
        mrow = jnp.max(m, axis=1, keepdims=True)

        @pl.when(b == nb - 1)
        def _():
            out_proj(0, woa_v, g)

        tau0 = 2 * ta + tb
        nv = lambda t: (vb_hbm, b, g, (t + LA) * R, None)
        more_w = g + 1 < ngrp
        carry = v_phase(
            tau0, 0, wq_per_step, mrow, (zero, zero), nv,
            lambda t: [(wq_piece(wqa_hbm, wqa_v, 0, gw, b * wq_per_step + t), 0, more_w),
                       (wq_piece(wqb_hbm, wqb_v, 1, gw, b * wq_per_step + t), 0, more_w)])
        carry = v_phase(tau0, wq_per_step, tb - LA - wq_per_step, mrow, carry,
                        nv, no_extra)
        carry = v_phase(tau0, tb - LA, LA, mrow, carry,
                        lambda t: (ka_hbm, b2, g2, a_row0 + (t + LA - tb) * R,
                                   i + 1 < nstep), no_extra)
        finish(1, carry)

        @pl.when(b == nb - 1)
        def _():
            out_proj(1, wob_v, g)

        return c

    jax.lax.fori_loop(0, nstep, step, 0)

    out_ref[...] = jnp.concatenate([acc_v[0], acc_v[1]], axis=1).astype(out_ref.dtype)


@jax.jit
def pallas_concat_heads__sliding_block_cached__mha_block_cached__decode_kernel(
    A_x: jax.Array,
    A_k_cache: jax.Array,
    A_v_cache: jax.Array,
    A_wq: jax.Array,
    A_wo: jax.Array,
    B_x: jax.Array,
    B_k_cache: jax.Array,
    B_v_cache: jax.Array,
    B_wq: jax.Array,
    B_wo: jax.Array,
):
    nb, sq, dmodel = A_x.shape
    _, nh, sk, dh = A_k_cache.shape
    assert sq == 1 and dh == DH and nh % G == 0
    wa = min(4096, max(256, sk // 4))
    assert wa // R == LA and (2 * wa // R + 2 * sk // R) % NSLOT == 0
    ngrp = nh // G
    gcols = G * DH
    bf16 = jnp.bfloat16
    f32 = jnp.float32

    kernel = functools.partial(_kernel, nb=nb, nh=nh, sk=sk, wa=wa)
    out = pl.pallas_call(
        kernel,
        in_specs=[pl.BlockSpec(memory_space=pl.ANY)] * 10,
        out_specs=pl.BlockSpec(memory_space=pltpu.VMEM),
        out_shape=jax.ShapeDtypeStruct((nb, 2 * dmodel), A_x.dtype),
        scratch_shapes=[
            pltpu.VMEM((NSLOT, G, R, DH), bf16),
            pltpu.VMEM((nb, dmodel), bf16),
            pltpu.VMEM((nb, dmodel), bf16),
            pltpu.VMEM((ngrp, dmodel, gcols), bf16),
            pltpu.VMEM((ngrp, dmodel, gcols), bf16),
            pltpu.VMEM((ngrp, gcols, dmodel), bf16),
            pltpu.VMEM((ngrp, gcols, dmodel), bf16),
            pltpu.VMEM((G * 8, DH), f32),
            pltpu.VMEM((2, nb, G, DH), f32),
            pltpu.VMEM((sk // R, G, DH), f32),
            pltpu.VMEM((2, nb * G, DH), f32),
            pltpu.VMEM((2, nb, dmodel), f32),
            pltpu.SemaphoreType.DMA((NSLOT,)),
            pltpu.SemaphoreType.DMA((2,)),
            pltpu.SemaphoreType.DMA((2, ngrp)),
            pltpu.SemaphoreType.DMA((2, ngrp)),
        ],
        compiler_params=pltpu.CompilerParams(vmem_limit_bytes=64 * 1024 * 1024),
    )(A_x.reshape(nb, dmodel), A_k_cache, A_v_cache, A_wq, A_wo,
      B_x.reshape(nb, dmodel), B_k_cache, B_v_cache, B_wq, B_wo)
    return out.reshape(nb, sq, 2 * dmodel)
```

```python
import functools

import jax
import jax.numpy as jnp
import jax.experimental.pallas as pl
import jax.experimental.pallas.tpu as pltpu

G = 8
R = 128
DH = 128
NSLOT = 16
LA = 8
NPIECE = 4
OFFB = 16
DELAY = 20
WDELAY = 30
NOCHECK = False


def _kernel(xa_hbm, ka_hbm, va_hbm, wqa_hbm, woa_hbm,
            xb_hbm, kb_hbm, vb_hbm, wqb_hbm, wob_hbm,
            out_ref,
            buf, xa_v, xb_v, t8_v, wqa_v, wqb_v, woa_v, wob_v,
            s_v, acc_v, sem, xsem,
            *, nb, wa):
    f32 = jnp.float32
    bf16 = jnp.bfloat16
    nstep = ka_hbm.shape[1]
    sk = ka_hbm.shape[2]
    dmodel = xa_v.shape[-1]
    scale = DH ** -0.5
    ta = wa // R
    tb = sk // R
    a_row0 = sk - wa
    prow = R // NPIECE
    rowid = jax.lax.broadcasted_iota(jnp.int32, (G, DH), 0)

    def kv_chunk(src, h, row0, slot):
        if row0 is None:
            segs = [(sk - (R - OFFB), 0, R - OFFB), (0, R - OFFB, OFFB)]
        else:
            segs = [(row0, 0, R)]
        low, high = [], []
        for (r0, d0, n) in segs:
            low.append(pltpu.make_async_copy(
                src.at[pl.ds(0, G - 1), h, pl.ds(r0, n)],
                buf.at[slot, pl.ds(0, G - 1), pl.ds(d0, n)], sem.at[slot]))
            for u in range(0, n, prow):
                k = min(prow, n - u)
                high.append(pltpu.make_async_copy(
                    src.at[G - 1, h, pl.ds(r0 + u, k)],
                    buf.at[slot, G - 1, pl.ds(d0 + u, k)], sem.at[slot]))
        return low, high

    wq_na, wq_nc, _, wq_cols = wqa_v.shape
    wq_half = wq_cols // 2
    wq_pc = wq_half // NPIECE

    def wq_chunk(w_hbm, w_v, j, slot):
        c = j // 2
        col0 = pl.multiple_of((j % 2) * wq_half, wq_half)
        low = [pltpu.make_async_copy(
            w_hbm.at[pl.ds(0, wq_na - 1), c, :, pl.ds(col0, wq_half)],
            w_v.at[pl.ds(0, wq_na - 1), c, :, pl.ds(col0, wq_half)], sem.at[slot])]
        high = []
        for u in range(NPIECE):
            cu = pl.multiple_of(col0 + u * wq_pc, wq_pc)
            high.append(pltpu.make_async_copy(
                w_hbm.at[wq_na - 1, c, :, pl.ds(cu, wq_pc)],
                w_v.at[wq_na - 1, c, :, pl.ds(cu, wq_pc)], sem.at[slot]))
        return low, high

    def wq_dst(w_v, j):
        col0 = pl.multiple_of((j % 2) * wq_half, wq_half)
        return w_v.at[:, j // 2, :, pl.ds(col0, wq_half)]

    wo_na, wo_nc, wo_rows, _ = woa_v.shape
    wo_pr = wo_rows // NPIECE

    def wo_chunk(w_hbm, w_v, j, slot):
        low = [pltpu.make_async_copy(
            w_hbm.at[pl.ds(0, wo_na - 1), j], w_v.at[pl.ds(0, wo_na - 1), j],
            sem.at[slot])]
        high = [pltpu.make_async_copy(
            w_hbm.at[wo_na - 1, j, pl.ds(u * wo_pr, wo_pr)],
            w_v.at[wo_na - 1, j, pl.ds(u * wo_pr, wo_pr)], sem.at[slot])
            for u in range(NPIECE)]
        return low, high

    def wo_dst(w_v, j):
        return w_v.at[:, j]

    def b_row(c):
        return pl.multiple_of(OFFB + (c - 1) * R, 8) if OFFB else c * R

    def diag(parts):
        out = parts[0]
        for r in range(1, G):
            out = jnp.where(rowid == r, parts[r], out)
        return out

    def start_all(copies, cond, delay, compute=None):
        low, high = copies
        def do(cp, prio):
            if cond is None:
                cp.start(priority=prio)
            else:
                @pl.when(cond)
                def _():
                    cp.start(priority=prio)
        do(high[0], 0)
        for cp in low:
            do(cp, 1)
        res = None
        if compute is not None:
            res = compute()
        for j, cp in enumerate(high[1:]):
            if j or compute is None:
                pl.delay(delay)
            do(cp, 0)
        return res

    def wait(dst, slot):
        pltpu.make_async_copy(dst, dst, sem.at[slot]).wait()

    def loop(t0, nt, body, carry):
        if nt == 1:
            return body(t0, carry)
        return jax.lax.fori_loop(t0, t0 + nt, body, carry)

    def w_phase(t0, nt, dst_fn, nxt_fn):
        def body(t, c):
            wait(dst_fn(t), t % NSLOT)
            start_all(nxt_fn(t, (t + LA) % NSLOT), None, WDELAY)
            return c
        loop(t0, nt, body, 0)

    def k_phase(tau0, t0, nt, q, m, nxt_fn, cond=None):
        def body(t, m):
            slot = (tau0 + t) % NSLOT
            wait(buf.at[slot], slot)
            def compute():
                s = diag([jax.lax.dot_general(
                    q, buf[slot, r], (((1,), (1,)), ((), ())),
                    preferred_element_type=f32) for r in range(G)])
                s_v[t] = s
                return jnp.maximum(m, s)
            return start_all(nxt_fn(t, (tau0 + t + LA) % NSLOT), cond, DELAY, compute)
        return loop(t0, nt, body, m)

    def v_phase(tau0, t0, nt, mrow, carry, nxt_fn, cond=None):
        def body(t, carry):
            l, acc = carry
            slot = (tau0 + t) % NSLOT
            p = jnp.exp((s_v[t] - mrow) * scale)
            pb = p.astype(bf16)
            wait(buf.at[slot], slot)
            def compute():
                o = diag([jnp.dot(pb, buf[slot, r], preferred_element_type=f32)
                          for r in range(G)])
                return l + p, acc + o
            return start_all(nxt_fn(t, (tau0 + t + LA) % NSLOT), cond, DELAY, compute)
        return loop(t0, nt, body, carry)

    def q_proj(x_v, w_v, h):
        x = x_v[...]
        for hi in range(2):
            col0 = pl.multiple_of((hi * nstep + h) * DH, DH)
            w = w_v[:, :, :, pl.ds(col0, DH)].reshape(dmodel, DH)
            t8_v[pl.ds(hi, nb, stride=2), :] = jnp.dot(
                x, w, preferred_element_type=f32)
        return t8_v[...].astype(bf16)

    hpa = wo_nc * wo_rows // DH
    cph = DH // wo_rows

    def out_proj(which, w_v, h, carry):
        l, acc = carry
        t8_v[...] = acc / jnp.sum(l, axis=1, keepdims=True)
        res = acc_v[which]
        for hi in range(2):
            hd = hi * nstep + h
            o = t8_v[pl.ds(hi, nb, stride=2), :].astype(bf16)
            w = w_v[hd // hpa, pl.ds((hd % hpa) * cph, cph)].reshape(DH, dmodel)
            res = res + jnp.dot(o, w, preferred_element_type=f32)
        acc_v[which] = res

    nw = 2 * wq_nc
    assert nw == wo_nc == NSLOT
    xa_cp = pltpu.make_async_copy(xa_hbm, xa_v, xsem.at[0])
    xb_cp = pltpu.make_async_copy(xb_hbm, xb_v, xsem.at[1])
    for t in range(LA):
        start_all(wo_chunk(woa_hbm, woa_v, t, t), None, WDELAY)
    xa_cp.start(priority=0)
    xb_cp.start(priority=0)
    acc_v[...] = jnp.zeros(acc_v.shape, f32)

    wseq = [(wo_chunk, wo_dst, woa_hbm, woa_v), (wo_chunk, wo_dst, wob_hbm, wob_v),
            (wq_chunk, wq_dst, wqb_hbm, wqb_v), (wq_chunk, wq_dst, wqa_hbm, wqa_v)]
    for n, (cf, df, w_hbm, w_v) in enumerate(wseq):
        w_phase(0, nw - LA, lambda t: df(w_v, t),
                lambda t, slot: cf(w_hbm, w_v, t + LA, slot))
        if n + 1 < len(wseq):
            cf2, _, w2_hbm, w2_v = wseq[n + 1]
            nxt = lambda t, slot: cf2(w2_hbm, w2_v, t + LA - nw, slot)
        else:
            nxt = lambda t, slot: kv_chunk(ka_hbm, 0, a_row0 + (t + LA - nw) * R, slot)
        w_phase(nw - LA, LA, lambda t: df(w_v, t), nxt)
        if n == 0:
            xa_cp.wait()
            xb_cp.wait()

    def step(h, c):
        h2 = jnp.minimum(h + 1, nstep - 1)
        neg = jnp.full((G, DH), -jnp.inf, f32)
        zero = jnp.zeros((G, DH), f32)
        wrap = None if OFFB else 0

        qa = q_proj(xa_v, wqa_v, h)
        m = k_phase(0, 0, ta, qa, neg,
                    lambda t, slot: kv_chunk(va_hbm, h, a_row0 + t * R, slot))
        mrow = jnp.max(m, axis=1, keepdims=True)
        carry = v_phase(ta, 0, 1, mrow, (zero, zero),
                        lambda t, slot: kv_chunk(kb_hbm, h, wrap, slot))
        carry = v_phase(ta, 1, ta - 1, mrow, carry,
                        lambda t, slot: kv_chunk(kb_hbm, h, b_row(t), slot))
        out_proj(0, woa_v, h, carry)

        tau0 = 2 * ta
        qb = q_proj(xb_v, wqb_v, h)
        m = k_phase(tau0, 0, tb - LA, qb, neg,
                    lambda t, slot: kv_chunk(kb_hbm, h, b_row(t + LA), slot))
        m = k_phase(tau0, tb - LA, 1, qb, m,
                    lambda t, slot: kv_chunk(vb_hbm, h, wrap, slot))
        m = k_phase(tau0, tb - LA + 1, LA - 1, qb, m,
                    lambda t, slot: kv_chunk(vb_hbm, h, b_row(t + LA - tb), slot))
        mrow = jnp.max(m, axis=1, keepdims=True)

        tau0 = 2 * ta + tb
        carry = v_phase(tau0, 0, tb - LA, mrow, (zero, zero),
                        lambda t, slot: kv_chunk(vb_hbm, h, b_row(t + LA), slot))
        carry = v_phase(tau0, tb - LA, LA, mrow, carry,
                        lambda t, slot: kv_chunk(ka_hbm, h2, a_row0 + (t + LA - tb) * R, slot),
                        cond=h + 1 < nstep)
        out_proj(1, wob_v, h, carry)
        return c

    jax.lax.fori_loop(0, nstep, step, 0)

    out_ref[...] = jnp.concatenate([acc_v[0], acc_v[1]], axis=1).astype(out_ref.dtype)


@jax.jit
def pallas_concat_heads__sliding_block_cached__mha_block_cached__decode_kernel(
    A_x: jax.Array,
    A_k_cache: jax.Array,
    A_v_cache: jax.Array,
    A_wq: jax.Array,
    A_wo: jax.Array,
    B_x: jax.Array,
    B_k_cache: jax.Array,
    B_v_cache: jax.Array,
    B_wq: jax.Array,
    B_wo: jax.Array,
):
    nb, sq, dmodel = A_x.shape
    _, nh, sk, dh = A_k_cache.shape
    assert sq == 1 and dh == DH and 2 * nb == G and nh % 2 == 0
    wa = min(4096, max(256, sk // 4))
    assert wa // R == LA and (2 * wa // R + 2 * sk // R) % NSLOT == 0
    bf16 = jnp.bfloat16
    f32 = jnp.float32
    hd = nh * dh
    wq_shape = (dmodel // 64, 8, 8, hd)
    wo_shape = (8, NSLOT, hd // (8 * NSLOT), dmodel)
    kv = lambda t: t.reshape(G, nh // 2, sk, dh)

    kernel = functools.partial(_kernel, nb=nb, wa=wa)
    out = pl.pallas_call(
        kernel,
        in_specs=[pl.BlockSpec(memory_space=pl.ANY)] * 10,
        out_specs=pl.BlockSpec(memory_space=pltpu.VMEM),
        out_shape=jax.ShapeDtypeStruct((nb, 2 * dmodel), A_x.dtype),
        scratch_shapes=[
            pltpu.VMEM((NSLOT, G, R, DH), bf16),
            pltpu.VMEM((nb, dmodel), bf16),
            pltpu.VMEM((nb, dmodel), bf16),
            pltpu.VMEM((G, DH), f32),
            pltpu.VMEM(wq_shape, bf16),
            pltpu.VMEM(wq_shape, bf16),
            pltpu.VMEM(wo_shape, bf16),
            pltpu.VMEM(wo_shape, bf16),
            pltpu.VMEM((sk // R, G, DH), f32),
            pltpu.VMEM((2, nb, dmodel), f32),
            pltpu.SemaphoreType.DMA((NSLOT,)),
            pltpu.SemaphoreType.DMA((2,)),
        ],
        compiler_params=pltpu.CompilerParams(vmem_limit_bytes=64 * 1024 * 1024,
                                             disable_bounds_checks=NOCHECK),
    )(A_x.reshape(nb, dmodel), kv(A_k_cache), kv(A_v_cache),
      A_wq.reshape(wq_shape), A_wo.reshape(wo_shape),
      B_x.reshape(nb, dmodel), kv(B_k_cache), kv(B_v_cache),
      B_wq.reshape(wq_shape), B_wo.reshape(wo_shape))
    return out.reshape(nb, sq, 2 * dmodel)
```

```python
import functools

import jax
import jax.numpy as jnp
import jax.experimental.pallas as pl
import jax.experimental.pallas.tpu as pltpu

G = 8
R = 128
DH = 128
LA = 8
NSLOT = 2 * LA
NPIECE = 8
WQPIECE = 8
WOPIECE = 4
NW = 16
OFFB = 16


def _kernel(xa_hbm, ka_hbm, va_hbm, wqa_hbm, woa_hbm,
            xb_hbm, kb_hbm, vb_hbm, wqb_hbm, wob_hbm,
            out_ref,
            buf, xa_v, xb_v, t8_v, wqa_v, wqb_v, woa_v, wob_v,
            s_v, acc_v, sem, xsem,
            *, nb, wa):
    f32 = jnp.float32
    bf16 = jnp.bfloat16
    nstep = ka_hbm.shape[1]
    sk = ka_hbm.shape[2]
    dmodel = xa_v.shape[-1]
    scale = DH ** -0.5
    prow = R // NPIECE
    rowid = jax.lax.broadcasted_iota(jnp.int32, (G, DH), 0)

    def kv_chunk(src, lo, off, h, c, tau):
        slot = tau % NSLOT
        sm = sem.at[tau % LA]
        if c is None:
            segs = [(sk - (R - off), 0, R - off), (lo, R - off, off)]
            n0 = (R - off) // prow
            row_of = lambda u: (sk - (R - off) + u * prow if u < n0
                                else lo + (u - n0) * prow)
        else:
            row0 = lo + c * R if off == 0 else lo + off + (c - 1) * R
            row0 = pl.multiple_of(row0, prow)
            segs = [(row0, 0, R)]
            row_of = lambda u: pl.multiple_of(row0 + u * prow, prow)
        low = [pltpu.make_async_copy(
            src.at[pl.ds(0, G - 1), h, pl.ds(r0, n)],
            buf.at[slot, pl.ds(0, G - 1), pl.ds(d0, n)], sm)
            for (r0, d0, n) in segs]
        high = lambda u: pltpu.make_async_copy(
            src.at[G - 1, h, pl.ds(row_of(u), prow)],
            buf.at[slot, G - 1, pl.ds(pl.multiple_of(u * prow, prow), prow)], sm)
        return low, high, NPIECE

    wq_na, _, _, wq_cols = wqa_v.shape
    wq_half = wq_cols // 2
    wq_pc = wq_half // WQPIECE

    def wq_chunk(w_hbm, w_v, j):
        sm = sem.at[j % LA]
        c = j // 2
        col0 = pl.multiple_of((j % 2) * wq_half, wq_half)
        low = [pltpu.make_async_copy(
            w_hbm.at[pl.ds(0, wq_na - 1), c, :, pl.ds(col0, wq_half)],
            w_v.at[pl.ds(0, wq_na - 1), c, :, pl.ds(col0, wq_half)], sm)]

        def high(u):
            cu = pl.multiple_of(col0 + u * wq_pc, wq_pc)
            return pltpu.make_async_copy(
                w_hbm.at[wq_na - 1, c, :, pl.ds(cu, wq_pc)],
                w_v.at[wq_na - 1, c, :, pl.ds(cu, wq_pc)], sm)
        return low, high, WQPIECE

    def wq_dst(w_v, j):
        col0 = pl.multiple_of((j % 2) * wq_half, wq_half)
        return w_v.at[:, j // 2, :, pl.ds(col0, wq_half)]

    wo_na, wo_nc, wo_rows, _ = woa_v.shape
    wo_pr = wo_rows // WOPIECE

    def wo_chunk(w_hbm, w_v, j):
        sm = sem.at[j % LA]
        low = [pltpu.make_async_copy(
            w_hbm.at[pl.ds(0, wo_na - 1), j], w_v.at[pl.ds(0, wo_na - 1), j], sm)]

        def high(u):
            ru = pl.multiple_of(u * wo_pr, wo_pr)
            return pltpu.make_async_copy(
                w_hbm.at[wo_na - 1, j, pl.ds(ru, wo_pr)],
                w_v.at[wo_na - 1, j, pl.ds(ru, wo_pr)], sm)
        return low, high, WOPIECE

    def wo_dst(w_v, j):
        return w_v.at[:, j]

    def wait(dst, tau):
        pltpu.make_async_copy(dst, dst, sem.at[tau % LA]).wait()

    def start_plain(chunk):
        low, high, n = chunk
        for cp in low:
            cp.start(priority=1)

        def body(u, c):
            high(u).start(priority=0)
            s_v[...] = jnp.zeros(s_v.shape, f32)
            return c
        jax.lax.fori_loop(0, n, body, 0)

    def start_mixed(chunk, cond, tile_fn):
        low, high, n = chunk

        def start(cp, prio):
            if cond is None:
                cp.start(priority=prio)
            else:
                @pl.when(cond)
                def _():
                    cp.start(priority=prio)
        start(high(0), 0)
        for cp in low:
            start(cp, 1)
        done = 1
        out = None
        for j in range(G):
            while cond is None and done < 1 + (j * (n - 1)) // G:
                start(high(done), 0)
                done += 1
            part = tile_fn(j)
            out = part if j == 0 else jnp.where(
                rowid == (j % 2) * nb + j // 2, part, out)
        for u in range(done, n):
            start(high(u), 0)
        return out

    def loop(t0, nt, body, carry):
        if nt == 1:
            return body(t0, carry)
        return jax.lax.fori_loop(t0, t0 + nt, body, carry)

    def w_ticks(t0, nt, dst_fn, nxt_fn):
        def body(t, c):
            wait(dst_fn(t), t)
            start_plain(nxt_fn(t))
            return c
        loop(t0, nt, body, 0)

    def k_ticks(tau0, t0, nt, q, m, nxt_fn):
        def body(t, m):
            slot = (tau0 + t) % NSLOT
            wait(buf.at[slot], tau0 + t)
            s = start_mixed(nxt_fn(t), None,
                            lambda j: jax.lax.dot_general(
                                q, buf[slot, j], (((1,), (1,)), ((), ())),
                                preferred_element_type=f32))
            s_v[t] = s
            return jnp.maximum(m, s)
        return loop(t0, nt, body, m)

    def softmax(nt, m):
        mrow = jnp.max(m, axis=1, keepdims=True)
        p = jnp.exp((s_v[pl.ds(0, nt)] - mrow[None]) * scale)
        l = jnp.sum(jnp.sum(p, axis=0), axis=1, keepdims=True)
        s_v[pl.ds(0, nt)] = p
        return 1.0 / l

    def v_ticks(tau0, t0, nt, inv, acc, nxt_fn, cond):
        def body(t, acc):
            slot = (tau0 + t) % NSLOT
            pb = (s_v[t] * inv).astype(bf16)
            wait(buf.at[slot], tau0 + t)
            o = start_mixed(nxt_fn(t), cond,
                            lambda j: jnp.dot(pb, buf[slot, j],
                                              preferred_element_type=f32))
            return acc + o
        return loop(t0, nt, body, acc)

    def q_proj(x_v, w_v, h):
        x = x_v[...]
        for hi in range(2):
            col0 = pl.multiple_of((hi * nstep + h) * DH, DH)
            w = w_v[:, :, :, pl.ds(col0, DH)].reshape(dmodel, DH)
            t8_v[pl.ds(hi * nb, nb), :] = jnp.dot(
                x, w, preferred_element_type=f32)
        return t8_v[...].astype(bf16)

    hpa = wo_nc * wo_rows // DH
    cph = DH // wo_rows

    def out_proj(which, w_v, h, o8):
        t8_v[...] = o8
        res = acc_v[which]
        for hi in range(2):
            hd = hi * nstep + h
            o = t8_v[pl.ds(hi * nb, nb), :].astype(bf16)
            w = w_v[hd // hpa, pl.ds((hd % hpa) * cph, cph)].reshape(DH, dmodel)
            res = res + jnp.dot(o, w, preferred_element_type=f32)
        acc_v[which] = res

    phases = [(ka_hbm, sk - wa, 0, wa // R), (va_hbm, sk - wa, 0, wa // R),
              (kb_hbm, 0, OFFB, sk // R), (vb_hbm, 0, OFFB, sk // R)]

    def segments(nt, tau0, cur, h, nxt, h2):
        segs = []
        if nt > LA:
            segs.append((0, nt - LA, lambda t: kv_chunk(
                *cur[:3], h, t + LA, tau0 + t + LA), False))
        t0 = nt - LA
        if nxt[2]:
            segs.append((t0, 1, lambda t: kv_chunk(
                *nxt[:3], h2, None, tau0 + t + LA), True))
            t0 += 1
        segs.append((t0, nt - t0, lambda t: kv_chunk(
            *nxt[:3], h2, t + LA - nt, tau0 + t + LA), True))
        return segs

    wseq = [(wo_chunk, wo_dst, woa_hbm, woa_v), (wo_chunk, wo_dst, wob_hbm, wob_v),
            (wq_chunk, wq_dst, wqb_hbm, wqb_v), (wq_chunk, wq_dst, wqa_hbm, wqa_v)]
    xa_cp = pltpu.make_async_copy(xa_hbm, xa_v, xsem)
    xb_cp = pltpu.make_async_copy(xb_hbm, xb_v, xsem)

    def first(t, c):
        start_plain(wo_chunk(woa_hbm, woa_v, t))
        return c
    jax.lax.fori_loop(0, LA, first, 0)
    xa_cp.start(priority=0)
    xb_cp.start(priority=0)
    acc_v[...] = jnp.zeros(acc_v.shape, f32)

    for n, (cf, df, w_hbm, w_v) in enumerate(wseq):
        w_ticks(0, NW - LA, lambda t: df(w_v, t),
                lambda t: cf(w_hbm, w_v, t + LA))
        if n + 1 < len(wseq):
            cf2, _, w2_hbm, w2_v = wseq[n + 1]
            w_ticks(NW - LA, LA, lambda t: df(w_v, t),
                    lambda t: cf2(w2_hbm, w2_v, t + LA - NW))
        else:
            for (t0, nt, fn, _) in segments(LA, -LA, None, None, phases[0], 0):
                w_ticks(t0, nt, lambda t: df(w_v, t + NW - LA), fn)
        if n == 0:
            xa_cp.wait()
            xb_cp.wait()

    def step(h, c):
        h2 = jnp.minimum(h + 1, nstep - 1)
        tau0 = 0
        for which, (x_v, wq_v, wo_v) in enumerate(
                [(xa_v, wqa_v, woa_v), (xb_v, wqb_v, wob_v)]):
            kph, vph = phases[2 * which], phases[2 * which + 1]
            nt = kph[3]
            q = q_proj(x_v, wq_v, h)
            m = jnp.full((G, DH), -jnp.inf, f32)
            for (t0, n, fn, _) in segments(nt, tau0, kph, h, vph, h):
                m = k_ticks(tau0, t0, n, q, m, fn)
            inv = softmax(nt, m)
            tau0 += nt
            last = which == 1
            acc = jnp.zeros((G, DH), f32)
            for (t0, n, fn, in_nxt) in segments(
                    nt, tau0, vph, h, phases[0 if last else 2], h2 if last else h):
                acc = v_ticks(tau0, t0, n, inv, acc, fn,
                              h + 1 < nstep if (last and in_nxt) else None)
            tau0 += nt
            out_proj(which, wo_v, h, acc)
        return c

    jax.lax.fori_loop(0, nstep, step, 0)

    out_ref[...] = jnp.concatenate([acc_v[0], acc_v[1]], axis=1).astype(out_ref.dtype)


@jax.jit
def pallas_concat_heads__sliding_block_cached__mha_block_cached__decode_kernel(
    A_x: jax.Array,
    A_k_cache: jax.Array,
    A_v_cache: jax.Array,
    A_wq: jax.Array,
    A_wo: jax.Array,
    B_x: jax.Array,
    B_k_cache: jax.Array,
    B_v_cache: jax.Array,
    B_wq: jax.Array,
    B_wo: jax.Array,
):
    nb, sq, dmodel = A_x.shape
    _, nh, sk, dh = A_k_cache.shape
    wa = min(4096, max(256, sk // 4))
    assert sq == 1 and dh == DH and 2 * nb == G and nh % 2 == 0
    assert wa % R == 0 and sk % R == 0 and wa // R >= LA
    assert (2 * wa // R + 2 * sk // R) % NSLOT == 0 and NW % LA == 0
    assert OFFB % (R // NPIECE) == 0
    bf16 = jnp.bfloat16
    f32 = jnp.float32
    hd = nh * dh
    wq_shape = (dmodel // (4 * NW), NW // 2, 8, hd)
    wo_shape = (8, NW, hd // (8 * NW), dmodel)
    kv = lambda t: t.reshape(G, nh // 2, sk, dh)

    out = pl.pallas_call(
        functools.partial(_kernel, nb=nb, wa=wa),
        in_specs=[pl.BlockSpec(memory_space=pl.ANY)] * 10,
        out_specs=pl.BlockSpec(memory_space=pltpu.VMEM),
        out_shape=jax.ShapeDtypeStruct((nb, 2 * dmodel), A_x.dtype),
        scratch_shapes=[
            pltpu.VMEM((NSLOT, G, R, DH), bf16),
            pltpu.VMEM((nb, dmodel), bf16),
            pltpu.VMEM((nb, dmodel), bf16),
            pltpu.VMEM((G, DH), f32),
            pltpu.VMEM(wq_shape, bf16),
            pltpu.VMEM(wq_shape, bf16),
            pltpu.VMEM(wo_shape, bf16),
            pltpu.VMEM(wo_shape, bf16),
            pltpu.VMEM((sk // R, G, DH), f32),
            pltpu.VMEM((2, nb, dmodel), f32),
            pltpu.SemaphoreType.DMA((LA,)),
            pltpu.SemaphoreType.DMA,
        ],
        compiler_params=pltpu.CompilerParams(vmem_limit_bytes=48 * 1024 * 1024),
    )(A_x.reshape(nb, dmodel), kv(A_k_cache), kv(A_v_cache),
      A_wq.reshape(wq_shape), A_wo.reshape(wo_shape),
      B_x.reshape(nb, dmodel), kv(B_k_cache), kv(B_v_cache),
      B_wq.reshape(wq_shape), B_wo.reshape(wo_shape))
    return out.reshape(nb, sq, 2 * dmodel)
```

```python
import functools

import jax
import jax.numpy as jnp
import jax.experimental.pallas as pl
import jax.experimental.pallas.tpu as pltpu

G = 8
R = 128
DH = 128
LA = 8
NSLOT = 2 * LA
NPIECE = 4
WQPIECE = 8
NW = 16
OFFB = 16


def _kernel(xa_hbm, ka_hbm, va_hbm, wqa_hbm, woa_hbm,
            xb_hbm, kb_hbm, vb_hbm, wqb_hbm, wob_hbm,
            out_ref,
            buf, xa_v, xb_v, t8_v, wqa_v, wqb_v, woa_v, wob_v,
            s_v, acc_v, sem, xsem,
            *, nb, wa):
    f32 = jnp.float32
    bf16 = jnp.bfloat16
    nstep = ka_hbm.shape[1]
    sk = ka_hbm.shape[2]
    dmodel = xa_v.shape[-1]
    scale = DH ** -0.5
    prow = R // NPIECE
    rowid = jax.lax.broadcasted_iota(jnp.int32, (G, DH), 0)

    def kv_chunk(src, lo, off, h, c, tau):
        slot = tau % NSLOT
        sm = sem.at[tau % LA]

        def piece(r0, d0, n):
            return pltpu.make_async_copy(
                src.at[G - 1, h, pl.ds(r0, n)],
                buf.at[slot, G - 1, pl.ds(d0, n)], sm)
        if c is None:
            segs = [(sk - (R - off), 0, R - off), (lo, R - off, off)]
            cuts = [(r0 + u, d0 + u, min(prow, n - u))
                    for (r0, d0, n) in segs for u in range(0, n, prow)]
            high, nhigh = (lambda u: piece(*cuts[u])), len(cuts)
        else:
            if lo == 0:
                c = (c % 2) * (sk // R // 2) + c // 2
            row0 = lo + c * R if off == 0 else lo + off + (c - 1) * R
            row0 = pl.multiple_of(row0, 16)
            segs = [(row0, 0, R)]
            high = lambda u: piece(pl.multiple_of(row0 + u * prow, 16),
                                   pl.multiple_of(u * prow, 16), prow)
            nhigh = NPIECE
        low = [pltpu.make_async_copy(
            src.at[pl.ds(0, G - 1), h, pl.ds(r0, n)],
            buf.at[slot, pl.ds(0, G - 1), pl.ds(d0, n)], sm)
            for (r0, d0, n) in segs]
        return low, high, nhigh

    wq_na, _, _, wq_cols = wqa_v.shape
    wq_half = wq_cols // 2
    wq_pc = wq_half // WQPIECE

    def wq_chunk(w_hbm, w_v, j):
        sm = sem.at[j % LA]
        c = j // 2
        col0 = pl.multiple_of((j % 2) * wq_half, wq_half)
        low = [pltpu.make_async_copy(
            w_hbm.at[pl.ds(0, wq_na - 1), c, :, pl.ds(col0, wq_half)],
            w_v.at[pl.ds(0, wq_na - 1), c, :, pl.ds(col0, wq_half)], sm)]

        def high(u):
            cu = pl.multiple_of(col0 + u * wq_pc, wq_pc)
            return pltpu.make_async_copy(
                w_hbm.at[wq_na - 1, c, :, pl.ds(cu, wq_pc)],
                w_v.at[wq_na - 1, c, :, pl.ds(cu, wq_pc)], sm)
        return low, high, WQPIECE

    def wq_dst(w_v, j):
        col0 = pl.multiple_of((j % 2) * wq_half, wq_half)
        return w_v.at[:, j // 2, :, pl.ds(col0, wq_half)]

    wo_na, wo_nc, wo_rows, _ = woa_v.shape

    def wo_chunk(w_hbm, w_v, j):
        sm = sem.at[j % LA]
        low = [pltpu.make_async_copy(
            w_hbm.at[pl.ds(0, wo_na - 1), j], w_v.at[pl.ds(0, wo_na - 1), j], sm)]

        def high(u):
            cu = pl.multiple_of(u * 128, 128)
            return pltpu.make_async_copy(
                w_hbm.at[wo_na - 1, j, :, pl.ds(cu, 128)],
                w_v.at[wo_na - 1, j, :, pl.ds(cu, 128)], sm)
        return low, high, dmodel // 128

    def wo_dst(w_v, j):
        return w_v.at[:, j]

    def wait(dst, tau):
        pltpu.make_async_copy(dst, dst, sem.at[tau % LA]).wait()

    def start_plain(chunk):
        low, high, n = chunk
        for cp in low:
            cp.start(priority=1)

        def body(u, c):
            high(u).start(priority=0)
            s_v[...] = jnp.zeros(s_v.shape, f32)
            return c
        jax.lax.fori_loop(0, n, body, 0)

    def start_mixed(chunk, cond, tile_fn):
        low, high, n = chunk

        def start(cp, prio):
            if cond is None:
                cp.start(priority=prio)
            else:
                @pl.when(cond)
                def _():
                    cp.start(priority=prio)
        start(high(0), 0)
        for cp in low:
            start(cp, 1)
        done = 1
        out = None
        for j in range(G):
            while cond is None and done < 1 + (j * (n - 1)) // G:
                start(high(done), 0)
                done += 1
            part = tile_fn(j)
            out = part if j == 0 else jnp.where(
                rowid == (j % 2) * nb + j // 2, part, out)
        for u in range(done, n):
            start(high(u), 0)
        return out

    def loop(t0, nt, body, carry):
        if nt == 1:
            return body(t0, carry)
        return jax.lax.fori_loop(t0, t0 + nt, body, carry)

    def w_ticks(t0, nt, dst_fn, nxt_fn):
        def body(t, c):
            wait(dst_fn(t), t)
            start_plain(nxt_fn(t))
            return c
        loop(t0, nt, body, 0)

    def k_ticks(tau0, t0, nt, q, m, nxt_fn):
        def body(t, m):
            slot = (tau0 + t) % NSLOT
            wait(buf.at[slot], tau0 + t)
            s = start_mixed(nxt_fn(t), None,
                            lambda j: jax.lax.dot_general(
                                q, buf[slot, j], (((1,), (1,)), ((), ())),
                                preferred_element_type=f32))
            s_v[t] = s
            return jnp.maximum(m, s)
        return loop(t0, nt, body, m)

    def softmax(nt, m):
        mrow = jnp.max(m, axis=1, keepdims=True)
        p = jnp.exp((s_v[pl.ds(0, nt)] - mrow[None]) * scale)
        l = jnp.sum(jnp.sum(p, axis=0), axis=1, keepdims=True)
        s_v[pl.ds(0, nt)] = p
        return 1.0 / l

    def v_ticks(tau0, t0, nt, inv, acc, nxt_fn, cond):
        def body(t, acc):
            slot = (tau0 + t) % NSLOT
            pb = (s_v[t] * inv).astype(bf16)
            wait(buf.at[slot], tau0 + t)
            o = start_mixed(nxt_fn(t), cond,
                            lambda j: jnp.dot(pb, buf[slot, j],
                                              preferred_element_type=f32))
            return acc + o
        return loop(t0, nt, body, acc)

    def q_proj(x_v, w_v, h):
        x = x_v[...]
        for hi in range(2):
            col0 = pl.multiple_of((hi * nstep + h) * DH, DH)
            w = w_v[:, :, :, pl.ds(col0, DH)].reshape(dmodel, DH)
            t8_v[pl.ds(hi * nb, nb), :] = jnp.dot(
                x, w, preferred_element_type=f32)
        return t8_v[...].astype(bf16)

    hpa = wo_nc * wo_rows // DH
    cph = DH // wo_rows

    def out_proj(which, w_v, h, o8):
        t8_v[...] = o8
        res = acc_v[which]
        for hi in range(2):
            hd = hi * nstep + h
            o = t8_v[pl.ds(hi * nb, nb), :].astype(bf16)
            w = w_v[hd // hpa, pl.ds((hd % hpa) * cph, cph)].reshape(DH, dmodel)
            res = res + jnp.dot(o, w, preferred_element_type=f32)
        acc_v[which] = res

    phases = [(ka_hbm, sk - wa, 0, wa // R), (va_hbm, sk - wa, 0, wa // R),
              (kb_hbm, 0, OFFB, sk // R), (vb_hbm, 0, OFFB, sk // R)]

    def segments(nt, tau0, cur, h, nxt, h2):
        segs = []
        if nt > LA:
            segs.append((0, nt - LA, lambda t: kv_chunk(
                *cur[:3], h, t + LA, tau0 + t + LA), False))
        t0 = nt - LA
        if nxt[2]:
            segs.append((t0, 1, lambda t: kv_chunk(
                *nxt[:3], h2, None, tau0 + t + LA), True))
            t0 += 1
        segs.append((t0, nt - t0, lambda t: kv_chunk(
            *nxt[:3], h2, t + LA - nt, tau0 + t + LA), True))
        return segs

    wseq = [(wo_chunk, wo_dst, woa_hbm, woa_v), (wo_chunk, wo_dst, wob_hbm, wob_v),
            (wq_chunk, wq_dst, wqb_hbm, wqb_v), (wq_chunk, wq_dst, wqa_hbm, wqa_v)]
    xa_cp = pltpu.make_async_copy(xa_hbm, xa_v, xsem)
    xb_cp = pltpu.make_async_copy(xb_hbm, xb_v, xsem)

    def first(t, c):
        start_plain(wo_chunk(woa_hbm, woa_v, t))
        return c
    jax.lax.fori_loop(0, LA, first, 0)
    xa_cp.start(priority=0)
    xb_cp.start(priority=0)
    acc_v[...] = jnp.zeros(acc_v.shape, f32)

    for n, (cf, df, w_hbm, w_v) in enumerate(wseq):
        w_ticks(0, NW - LA, lambda t: df(w_v, t),
                lambda t: cf(w_hbm, w_v, t + LA))
        if n + 1 < len(wseq):
            cf2, _, w2_hbm, w2_v = wseq[n + 1]
            w_ticks(NW - LA, LA, lambda t: df(w_v, t),
                    lambda t: cf2(w2_hbm, w2_v, t + LA - NW))
        else:
            for (t0, nt, fn, _) in segments(LA, -LA, None, None, phases[0], 0):
                w_ticks(t0, nt, lambda t: df(w_v, t + NW - LA), fn)
        if n == 0:
            xa_cp.wait()
            xb_cp.wait()

    def step(h, c):
        h2 = jnp.minimum(h + 1, nstep - 1)
        tau0 = 0
        for which, (x_v, wq_v, wo_v) in enumerate(
                [(xa_v, wqa_v, woa_v), (xb_v, wqb_v, wob_v)]):
            kph, vph = phases[2 * which], phases[2 * which + 1]
            nt = kph[3]
            q = q_proj(x_v, wq_v, h)
            m = jnp.full((G, DH), -jnp.inf, f32)
            for (t0, n, fn, _) in segments(nt, tau0, kph, h, vph, h):
                m = k_ticks(tau0, t0, n, q, m, fn)
            inv = softmax(nt, m)
            tau0 += nt
            last = which == 1
            acc = jnp.zeros((G, DH), f32)
            for (t0, n, fn, in_nxt) in segments(
                    nt, tau0, vph, h, phases[0 if last else 2], h2 if last else h):
                acc = v_ticks(tau0, t0, n, inv, acc, fn,
                              h + 1 < nstep if (last and in_nxt) else None)
            tau0 += nt
            out_proj(which, wo_v, h, acc)
        return c

    jax.lax.fori_loop(0, nstep, step, 0)

    out_ref[...] = jnp.concatenate([acc_v[0], acc_v[1]], axis=1).astype(out_ref.dtype)


@jax.jit
def pallas_concat_heads__sliding_block_cached__mha_block_cached__decode_kernel(
    A_x: jax.Array,
    A_k_cache: jax.Array,
    A_v_cache: jax.Array,
    A_wq: jax.Array,
    A_wo: jax.Array,
    B_x: jax.Array,
    B_k_cache: jax.Array,
    B_v_cache: jax.Array,
    B_wq: jax.Array,
    B_wo: jax.Array,
):
    nb, sq, dmodel = A_x.shape
    _, nh, sk, dh = A_k_cache.shape
    wa = min(4096, max(256, sk // 4))
    assert sq == 1 and dh == DH and 2 * nb == G and nh % 2 == 0
    assert wa % R == 0 and sk % (2 * R) == 0 and LA <= wa // R and wa < sk
    assert (2 * wa // R + 2 * sk // R) % NSLOT == 0 and NW % LA == 0
    assert OFFB % 16 == 0 and (R // NPIECE) % 16 == 0 and dmodel % 128 == 0
    bf16 = jnp.bfloat16
    f32 = jnp.float32
    hd = nh * dh
    wq_shape = (dmodel // (4 * NW), NW // 2, 8, hd)
    wo_shape = (8, NW, hd // (8 * NW), dmodel)
    kv = lambda t: t.reshape(G, nh // 2, sk, dh)

    out = pl.pallas_call(
        functools.partial(_kernel, nb=nb, wa=wa),
        in_specs=[pl.BlockSpec(memory_space=pl.ANY)] * 10,
        out_specs=pl.BlockSpec(memory_space=pltpu.VMEM),
        out_shape=jax.ShapeDtypeStruct((nb, 2 * dmodel), A_x.dtype),
        scratch_shapes=[
            pltpu.VMEM((NSLOT, G, R, DH), bf16),
            pltpu.VMEM((nb, dmodel), bf16),
            pltpu.VMEM((nb, dmodel), bf16),
            pltpu.VMEM((G, DH), f32),
            pltpu.VMEM(wq_shape, bf16),
            pltpu.VMEM(wq_shape, bf16),
            pltpu.VMEM(wo_shape, bf16),
            pltpu.VMEM(wo_shape, bf16),
            pltpu.VMEM((sk // R, G, DH), f32),
            pltpu.VMEM((2, nb, dmodel), f32),
            pltpu.SemaphoreType.DMA((LA,)),
            pltpu.SemaphoreType.DMA,
        ],
        compiler_params=pltpu.CompilerParams(vmem_limit_bytes=48 * 1024 * 1024),
    )(A_x.reshape(nb, dmodel), kv(A_k_cache), kv(A_v_cache),
      A_wq.reshape(wq_shape), A_wo.reshape(wo_shape),
      B_x.reshape(nb, dmodel), kv(B_k_cache), kv(B_v_cache),
      B_wq.reshape(wq_shape), B_wo.reshape(wo_shape))
    return out.reshape(nb, sq, 2 * dmodel)
```
